```python
import jax
import jax.numpy as jnp

def _softmax(x, axis=-1):
    return jax.nn.softmax(x, axis=axis)
def _gelu(x):
    return jax.nn.gelu(x, approximate=True)
def _silu(x):
    return jax.nn.silu(x)
def _sigmoid(x):
    return jax.nn.sigmoid(x)
def _layernorm(x, axis=-1, eps=1e-5):
    m = jnp.mean(x, axis=axis, keepdims=True)
    v = jnp.var(x, axis=axis, keepdims=True)
    return (x - m) / jnp.sqrt(v + eps)
def _scatter_add(tgt, idx, src, axis=0):
    return tgt.at[idx].add(src)
def _segment_sum(src, seg, n):
    return jax.ops.segment_sum(src, seg, n)
class _Rng:
    def __init__(self, key):
        self._k = key
    def _next(self):
        self._k, sub = jax.random.split(self._k)
        return sub
    def normal(self, shape):
        return jax.random.normal(self._next(), shape, dtype=jnp.bfloat16)
    def randint(self, lo, hi, shape):
        return jax.random.randint(self._next(), shape, lo, hi, dtype=jnp.int32)
    def uniform(self, shape, lo=0.0, hi=1.0):
        return jax.random.uniform(self._next(), shape, jnp.bfloat16, lo, hi)
    def permutation(self, n):
        return jax.random.permutation(self._next(), n)


kernel_name = 'recurrent_scan__sliding_block_cached__glu_gated_glu__decode'

def setup_inputs():
    _rng = _Rng(jax.random.key(int.from_bytes(__import__("os").urandom(4), "little")))
    _w = (lambda a: (lambda t: t.astype(jnp.bfloat16) if jnp.issubdtype(t.dtype, jnp.floating) else t)(jnp.asarray(a)))
    def _A_setup():
        B, Sq, D = 1, 1, 576
        Hq, Hkv, Sk, Dh = 32, 16, 65536, 128
        assert Hq % Hkv == 0, (Hq, Hkv)
        return {
            "x": _w((lambda *s: _rng.normal(s) * 0.05)(B, Sq, D)),
            "k_cache": _w((lambda *s: _rng.normal(s) * 0.05)(B, Hkv, Sk, Dh)),
            "v_cache": _w((lambda *s: _rng.normal(s) * 0.05)(B, Hkv, Sk, Dh)),
            "wq": _w((lambda *s: _rng.normal(s) * 0.05)(D, Hq * Dh) * (D ** -0.5)),
            "wo": _w((lambda *s: _rng.normal(s) * 0.05)(Hq * Dh, D) * ((Hq * Dh) ** -0.5)),
        }
    _A_in = _A_setup()

    def _B_setup():
        B, S, D, F = 1, 1, 576, 4608
        return {
            "x": _w((lambda *s: _rng.normal(s) * 0.05)(B, S, D)),
            "w_gate": _w((lambda *s: _rng.normal(s) * 0.05)(D, F)),
            "w_up": _w((lambda *s: _rng.normal(s) * 0.05)(D, F)),
            "w_down": _w((lambda *s: _rng.normal(s) * 0.05)(F, D)),
        }
    _B_in = _B_setup()

    return {
        "A_x": _A_in["x"],
        "A_k_cache": _A_in["k_cache"],
        "A_v_cache": _A_in["v_cache"],
        "A_wq": _A_in["wq"],
        "A_wo": _A_in["wo"],
        "B_x": _B_in["x"],
        "B_w_gate": _B_in["w_gate"],
        "B_w_up": _B_in["w_up"],
        "B_w_down": _B_in["w_down"],
    }

def reference(A_x, A_k_cache, A_v_cache, A_wq, A_wo, B_x, B_w_gate, B_w_up, B_w_down):
    def _A_ref(x, k_cache, v_cache, wq, wo):
        B, Sq, D = x.shape
        Hq, Dh = 32, 128
        Hkv, Sk = k_cache.shape[1], k_cache.shape[2]
        W = min(4096, max(256, Sk // 4))
        rep = Hq // Hkv
        q = (lambda x, *d: x.transpose(*d))((x @ wq).reshape(B, Sq, Hq, Dh), 0, 2, 1, 3)
        k = jnp.repeat(k_cache[:, :, Sk - W:, :], rep, axis=1)
        v = jnp.repeat(v_cache[:, :, Sk - W:, :], rep, axis=1)
        scores = jnp.einsum("bhqd,bhkd->bhqk", q, k) * (Dh ** -0.5)
        p = _softmax(scores, axis=-1)
        o = jnp.einsum("bhqk,bhkd->bhqd", p, v)
        return (lambda x, *d: x.transpose(*d))(o, 0, 2, 1, 3).reshape(B, Sq, Hq * Dh) @ wo

    def _B_ref(x, w_gate, w_up, w_down):
        g = jnp.einsum("bsd,df->bsf", x, w_gate)
        u = jnp.einsum("bsd,df->bsf", x, w_up)
        h = _sigmoid(g) * u
        return jnp.einsum("bsf,fd->bsd", h, w_down)

    x = A_x
    xn = _layernorm(x, axis=-1)
    s = _A_ref(xn, A_k_cache, A_v_cache, A_wq, A_wo)
    g = _silu(_B_ref(xn, B_w_gate, B_w_up, B_w_down))
    return x + s * g
```

```python
import jax
import jax.numpy as jnp
from jax import lax
import jax.experimental.pallas as pl
import jax.experimental.pallas.tpu as pltpu

_HQ = 32
_NN = (((1,), (0,)), ((), ()))
_NT = (((1,), (1,)), ((), ()))
_DEPTH = 4
_ROWS = 8
_WQ_CHUNKS = (1024,) * 4
_WO_CHUNKS = (1024,) * 4
_GU_CHUNKS = (1536,) * 3
_WD_CHUNKS = (1536, 1536, 1024, 384, 128)


def _sigmoid(x):
    return 1.0 / (1.0 + jnp.exp(-x))


@jax.jit
def pallas_recurrent_scan__sliding_block_cached__glu_gated_glu__decode_kernel(
    A_x: jax.Array,
    A_k_cache: jax.Array,
    A_v_cache: jax.Array,
    A_wq: jax.Array,
    A_wo: jax.Array,
    B_x: jax.Array,
    B_w_gate: jax.Array,
    B_w_up: jax.Array,
    B_w_down: jax.Array,
):
    del B_x
    _, _, D = A_x.shape
    _, Hkv, Sk, Dh = A_k_cache.shape
    W = min(4096, max(256, Sk // 4))
    F = B_w_gate.shape[1]
    cdt = A_wq.dtype
    f32 = jnp.float32
    assert _HQ == 2 * Hkv and Dh == 128
    assert sum(_WQ_CHUNKS) == sum(_WO_CHUNKS) == _HQ * Dh
    assert sum(_GU_CHUNKS) == sum(_WD_CHUNKS) == F

    def kernel(x_h, k_h, v_h, wq_h, wo_h, wg_h, wu_h, wd_h, o_ref,
               x_v, k_v, v_v, wq_v, wo_v, wg_v, wu_v, wd_v, sems):
        st = dict(q=[], o=[], h=[])
        steps = []

        def cols(src, dst, off, n):
            return src.at[:, pl.ds(off, n)], dst.at[:, pl.ds(off, n)]

        def dot(a, b, dims):
            return lax.dot_general(a, b, dims, preferred_element_type=f32)

        def layernorm():
            x = x_v[0].astype(f32)
            xc = x - jnp.mean(x, axis=-1, keepdims=True)
            var = jnp.mean(xc * xc, axis=-1, keepdims=True)
            xn = xc / jnp.sqrt(var + 1e-5)
            st["x"] = x
            st["xn"] = jnp.broadcast_to(xn, (_ROWS, D)).astype(cdt)
            st["s"] = jnp.zeros((_ROWS, D), f32)
            st["f"] = jnp.zeros((_ROWS, D), f32)

        def q_proj(off, n):
            q = dot(st["xn"], wq_v[:, pl.ds(off, n)], _NN)
            st["q"] += [q[:, j:j + Dh] for j in range(0, n, Dh)]

        def scores(h):
            row = lax.broadcasted_iota(jnp.int32, (_ROWS, Dh), 0)
            qh = jnp.where(row % 2 == 0, st["q"][2 * h], st["q"][2 * h + 1])
            s = dot(qh.astype(cdt), k_v[h], _NT) * (Dh ** -0.5)
            p = jnp.exp(s - jnp.max(s, axis=-1, keepdims=True))
            st["l"] = jnp.sum(p, axis=-1, keepdims=True)
            st["p"] = p.astype(cdt)

        def attend(h):
            o = dot(st["p"], v_v[h], _NN) / st["l"]
            st["o"] += [jnp.broadcast_to(o[r:r + 1], (_ROWS, Dh)).astype(cdt)
                        for r in range(2)]

        def o_proj(off, n):
            o = jnp.concatenate(st["o"][off // Dh:(off + n) // Dh], axis=1)
            st["s"] = st["s"] + dot(o, wo_v[:, pl.ds(off, n)], _NT)

        def gate(off, n):
            st["g"] = dot(st["xn"], wg_v[:, pl.ds(off, n)], _NN)

        def up(off, n):
            u = dot(st["xn"], wu_v[:, pl.ds(off, n)], _NN)
            hh = (_sigmoid(st["g"]) * u).astype(cdt)
            st["h"] += [hh[:, j:j + 128] for j in range(0, n, 128)]

        def down(off, n):
            hh = jnp.concatenate(st["h"][off // 128:(off + n) // 128], axis=1)
            st["f"] = st["f"] + dot(hh, wd_v[:, pl.ds(off, n)], _NT)

        def chunked(sizes):
            off = 0
            for n in sizes:
                yield off, n
                off += n

        for off, n in chunked(_WQ_CHUNKS):
            steps.append((*cols(wq_h, wq_v, off, n), [(q_proj, off, n)]))
        first = steps[0]
        steps[0] = (first[0], first[1], [])
        steps.insert(1, (x_h, x_v, [(layernorm,)] + first[2]))
        for h in range(Hkv):
            win = pl.ds(Sk - W, W)
            steps.append((k_h.at[0, h, win, :], k_v.at[h], [(scores, h)]))
            steps.append((v_h.at[0, h, win, :], v_v.at[h], [(attend, h)]))
        for off, n in chunked(_WO_CHUNKS):
            steps.append((*cols(wo_h, wo_v, off, n), [(o_proj, off, n)]))
        for off, n in chunked(_GU_CHUNKS):
            steps.append((*cols(wg_h, wg_v, off, n), [(gate, off, n)]))
            steps.append((*cols(wu_h, wu_v, off, n), [(up, off, n)]))
        for off, n in chunked(_WD_CHUNKS):
            steps.append((*cols(wd_h, wd_v, off, n), [(down, off, n)]))

        copies = [pltpu.make_async_copy(src, dst, sems.at[i % _DEPTH])
                  for i, (src, dst, _) in enumerate(steps)]
        for cp in copies[:_DEPTH]:
            cp.start()
        for i, (_, _, work) in enumerate(steps):
            copies[i].wait()
            if i + _DEPTH < len(copies):
                copies[i + _DEPTH].start()
            for fn, *args in work:
                fn(*args)

        f = st["f"][0:1]
        out = st["x"] + st["s"][0:1] * (f * _sigmoid(f))
        o_ref[0] = out.astype(o_ref.dtype)

    hbm = pl.BlockSpec(memory_space=pltpu.HBM)
    return pl.pallas_call(
        kernel,
        out_shape=jax.ShapeDtypeStruct(A_x.shape, A_x.dtype),
        in_specs=[hbm] * 8,
        out_specs=pl.BlockSpec(memory_space=pltpu.VMEM),
        scratch_shapes=[
            pltpu.VMEM(A_x.shape, A_x.dtype),
            pltpu.VMEM((Hkv, W, Dh), A_k_cache.dtype),
            pltpu.VMEM((Hkv, W, Dh), A_v_cache.dtype),
            pltpu.VMEM((D, _HQ * Dh), A_wq.dtype),
            pltpu.VMEM((D, _HQ * Dh), A_wo.dtype),
            pltpu.VMEM((D, F), B_w_gate.dtype),
            pltpu.VMEM((D, F), B_w_up.dtype),
            pltpu.VMEM((D, F), B_w_down.dtype),
            pltpu.SemaphoreType.DMA((_DEPTH,)),
        ],
        compiler_params=pltpu.CompilerParams(vmem_limit_bytes=100 * 2**20),
    )(A_x, A_k_cache, A_v_cache, A_wq, A_wo.T, B_w_gate, B_w_up, B_w_down.T)
```

```python
import jax
import jax.numpy as jnp
from jax import lax
import jax.experimental.pallas as pl
import jax.experimental.pallas.tpu as pltpu

_HQ = 32
_NN = (((1,), (0,)), ((), ()))
_NT = (((1,), (1,)), ((), ()))
_DEPTH = 3
_TAIL = 3
_ROWS = 8
_WQ_CHUNKS = (1024,) * 4
_GU_CHUNKS = (1536,) * 3
_WD_CHUNKS = (1536,) * 3
_WO_LAST_CHUNKS = (2048, 1024, 1024)


def _sigmoid(x):
    return 1.0 / (1.0 + jnp.exp(-x))


@jax.jit
def pallas_recurrent_scan__sliding_block_cached__glu_gated_glu__decode_kernel(
    A_x: jax.Array,
    A_k_cache: jax.Array,
    A_v_cache: jax.Array,
    A_wq: jax.Array,
    A_wo: jax.Array,
    B_x: jax.Array,
    B_w_gate: jax.Array,
    B_w_up: jax.Array,
    B_w_down: jax.Array,
):
    del B_x
    _, _, D = A_x.shape
    _, Hkv, Sk, Dh = A_k_cache.shape
    W = min(4096, max(256, Sk // 4))
    F = B_w_gate.shape[1]
    cdt = A_wq.dtype
    f32 = jnp.float32
    assert _HQ == 2 * Hkv and Dh == 128
    assert sum(_WQ_CHUNKS) == sum(_WO_LAST_CHUNKS) == _HQ * Dh
    assert sum(_GU_CHUNKS) == sum(_WD_CHUNKS) == F

    def kernel(x_h, k_h, v_h, wq_h, wo_h, wg_h, wu_h, wd_h, o_ref,
               x_v, k_v, v_v, wq_v, wo_v, wg_v, wu_v, wd_v, sems):
        st = dict(q=[], o=[], h=[], s={})
        steps = []

        def cols(src, dst, off, n):
            return src.at[:, pl.ds(off, n)], dst.at[:, pl.ds(off, n)]

        def dot(a, b, dims):
            return lax.dot_general(a, b, dims, preferred_element_type=f32)

        def layernorm():
            x = x_v[0].astype(f32)
            xc = x - jnp.mean(x, axis=-1, keepdims=True)
            var = jnp.mean(xc * xc, axis=-1, keepdims=True)
            xn = xc / jnp.sqrt(var + 1e-5)
            st["x"] = x
            st["xn"] = jnp.broadcast_to(xn, (_ROWS, D)).astype(cdt)
            st["f"] = jnp.zeros((_ROWS, D), f32)

        def q_proj(off, n):
            q = dot(st["xn"], wq_v[:, pl.ds(off, n)], _NN)
            st["q"] += [q[:, j:j + Dh] for j in range(0, n, Dh)]

        def scores(h):
            row = lax.broadcasted_iota(jnp.int32, (_ROWS, Dh), 0)
            qh = jnp.where(row % 2 == 0, st["q"][2 * h], st["q"][2 * h + 1])
            s = dot(qh.astype(cdt), k_v[h], _NT) * (Dh ** -0.5)
            p = jnp.exp(s - jnp.max(s, axis=-1, keepdims=True))
            st["l"] = jnp.sum(p, axis=-1, keepdims=True)
            st["p"] = p.astype(cdt)

        def attend(h):
            o = dot(st["p"], v_v[h], _NN) / st["l"]
            st["o"] += [jnp.broadcast_to(o[r:r + 1], (_ROWS, Dh)).astype(cdt)
                        for r in range(2)]

        def o_proj(r0, nr, off, n):
            o = jnp.concatenate(st["o"][off // Dh:(off + n) // Dh], axis=1)
            d = dot(o, wo_v[pl.ds(r0, nr), pl.ds(off, n)], _NT)
            st["s"][r0] = st["s"][r0] + d if r0 in st["s"] else d

        def gate(off, n):
            st["g"] = dot(st["xn"], wg_v[:, pl.ds(off, n)], _NN)

        def up(off, n):
            u = dot(st["xn"], wu_v[:, pl.ds(off, n)], _NN)
            hh = (_sigmoid(st["g"]) * u).astype(cdt)
            st["h"] += [hh[:, j:j + 128] for j in range(0, n, 128)]

        def down(off, n):
            hh = jnp.concatenate(st["h"][off // 128:(off + n) // 128], axis=1)
            st["f"] = st["f"] + dot(hh, wd_v[:, pl.ds(off, n)], _NT)

        def silu():
            f = st["f"][0:1]
            st["gate"] = f * _sigmoid(f)

        def chunked(sizes):
            off = 0
            for n in sizes:
                yield off, n
                off += n

        for off, n in chunked(_WQ_CHUNKS):
            steps.append((*cols(wq_h, wq_v, off, n), [(q_proj, off, n)]))
        first = steps[0]
        steps[0] = (first[0], first[1], [])
        steps.insert(1, (x_h, x_v, [(layernorm,)] + first[2]))
        for h in range(Hkv):
            win = pl.ds(Sk - W, W)
            steps.append((k_h.at[0, h, win, :], k_v.at[h], [(scores, h)]))
            steps.append((v_h.at[0, h, win, :], v_v.at[h], [(attend, h)]))
        for off, n in chunked(_GU_CHUNKS):
            steps.append((*cols(wg_h, wg_v, off, n), [(gate, off, n)]))
            steps.append((*cols(wu_h, wu_v, off, n), [(up, off, n)]))
        for off, n in chunked(_WD_CHUNKS):
            steps.append((*cols(wd_h, wd_v, off, n), [(down, off, n)]))

        steps[-1][2].append((silu,))
        last = (D - 1) // 128 * 128
        blocks = [(r0, 128, 0, _HQ * Dh) for r0 in range(0, last, 128)]
        blocks += [(last, D - last, off, n) for off, n in chunked(_WO_LAST_CHUNKS)]
        for r0, nr, off, n in blocks:
            idx = (pl.ds(r0, nr), pl.ds(off, n))
            steps.append((wo_h.at[idx], wo_v.at[idx], [(o_proj, r0, nr, off, n)]))

        tail = len(steps) - _TAIL
        start_after = [min(i, tail) - _DEPTH for i in range(len(steps))]
        copies = [
            pltpu.make_async_copy(
                src, dst, sems.at[i % _DEPTH if i <= tail else _DEPTH + i - tail - 1])
            for i, (src, dst, _) in enumerate(steps)]

        def start_copies(i):
            for cp, after in zip(copies, start_after):
                if max(after, -1) == i:
                    cp.start()

        start_copies(-1)
        for i, (_, _, work) in enumerate(steps):
            copies[i].wait()
            start_copies(i)
            for fn, *args in work:
                fn(*args)

        s = jnp.concatenate([st["s"][r0][0:1] for r0 in sorted(st["s"])], axis=1)
        o_ref[0] = (st["x"] + s * st["gate"]).astype(o_ref.dtype)

    hbm = pl.BlockSpec(memory_space=pltpu.HBM)
    return pl.pallas_call(
        kernel,
        out_shape=jax.ShapeDtypeStruct(A_x.shape, A_x.dtype),
        in_specs=[hbm] * 8,
        out_specs=pl.BlockSpec(memory_space=pltpu.VMEM),
        scratch_shapes=[
            pltpu.VMEM(A_x.shape, A_x.dtype),
            pltpu.VMEM((Hkv, W, Dh), A_k_cache.dtype),
            pltpu.VMEM((Hkv, W, Dh), A_v_cache.dtype),
            pltpu.VMEM((D, _HQ * Dh), A_wq.dtype),
            pltpu.VMEM((D, _HQ * Dh), A_wo.dtype),
            pltpu.VMEM((D, F), B_w_gate.dtype),
            pltpu.VMEM((D, F), B_w_up.dtype),
            pltpu.VMEM((D, F), B_w_down.dtype),
            pltpu.SemaphoreType.DMA((_DEPTH + _TAIL - 1,)),
        ],
        compiler_params=pltpu.CompilerParams(
            vmem_limit_bytes=100 * 2**20, disable_semaphore_checks=True),
    )(A_x, A_k_cache, A_v_cache, A_wq, A_wo.T, B_w_gate, B_w_up, B_w_down.T)
```
